```python
import os as _os
_os.environ.setdefault('JAX_PLATFORMS', 'cpu')
import jax
import jax.numpy as jnp

def _softmax(x, axis=-1):
    return jax.nn.softmax(x, axis=axis)

def _gelu(x):
    return jax.nn.gelu(x, approximate=True)

def _silu(x):
    return jax.nn.silu(x)

def _sigmoid(x):
    return jax.nn.sigmoid(x)

def _layernorm(x, axis=-1, eps=1e-05):
    m = jnp.mean(x, axis=axis, keepdims=True)
    v = jnp.var(x, axis=axis, keepdims=True)
    return (x - m) / jnp.sqrt(v + eps)

def _scatter_add(tgt, idx, src, axis=0):
    return tgt.at[idx].add(src)

def _segment_sum(src, seg, n):
    return jax.ops.segment_sum(src, seg, n)

class _Rng:

    def __init__(self, key):
        self._k = key

    def _next(self):
        self._k, sub = jax.random.split(self._k)
        return sub

    def normal(self, shape):
        return jax.random.normal(self._next(), shape, dtype=jnp.bfloat16)

    def randint(self, lo, hi, shape):
        return jax.random.randint(self._next(), shape, lo, hi, dtype=jnp.int32)

    def uniform(self, shape, lo=0.0, hi=1.0):
        return jax.random.uniform(self._next(), shape, jnp.bfloat16, lo, hi)

    def permutation(self, n):
        return jax.random.permutation(self._next(), n)
kernel_name = 'gated_mix__sliding_block__memory_aug_recurrent_mem_tr__prompt'

def setup_inputs():
    _rng = _Rng(jax.random.key(int.from_bytes(__import__("os").urandom(4), "little")))
    _w = lambda a: (lambda t: t.astype(jnp.bfloat16) if jnp.issubdtype(t.dtype, jnp.floating) else t)(jnp.asarray(a))

    def _A_setup():
        B, S, D = (1, 2048, 448)
        return {'x': _w((lambda *s: _rng.normal(s) * 0.05)(B, S, D)), 'wqkv': _w((lambda *s: _rng.normal(s) * 0.8)(D, 3 * D)), 'wo': _w((lambda *s: _rng.normal(s) * 0.05)(D, D))}
    _A_in = _A_setup()

    def _B_setup():
        B, S, Dm = (1, 2048, 448)
        H, Dh = (16, 256)
        M, seg = (8, 32)
        seg = min(seg, S)
        S = S // seg * seg
        return {'x': _w((lambda *s: _rng.normal(s) * 0.05)(B, S, Dm)), 'mem0': _w((lambda *s: _rng.normal(s) * 0.8)(B, M, Dm)), 'Wq': _w((lambda *s: _rng.normal(s) * 3.2)(Dm, H, Dh) * Dm ** (-0.5)), 'Wk': _w((lambda *s: _rng.normal(s) * 3.2)(Dm, H, Dh) * Dm ** (-0.5)), 'Wv': _w((lambda *s: _rng.normal(s) * 0.8)(Dm, H, Dh) * Dm ** (-0.5)), 'Wo': _w((lambda *s: _rng.normal(s) * 0.8)(H, Dh, Dm) * (H * Dh) ** (-0.5)), 'seg_len': seg}
    _B_in = _B_setup()
    return {'A_x': _A_in['x'], 'A_wqkv': _A_in['wqkv'], 'A_wo': _A_in['wo'], 'B_x': _B_in['x'], 'B_mem0': _B_in['mem0'], 'B_Wq': _B_in['Wq'], 'B_Wk': _B_in['Wk'], 'B_Wv': _B_in['Wv'], 'B_Wo': _B_in['Wo'], 'B_seg_len': _B_in['seg_len'], 'gate_w': _w((lambda *s: _rng.normal(s) * 0.05)(448) * 16.0)}

def reference(A_x, A_wqkv, A_wo, B_x, B_mem0, B_Wq, B_Wk, B_Wv, B_Wo, B_seg_len, gate_w):

    def _A_ref(x, wqkv, wo):
        B, S, D = x.shape
        H = 16
        Dh = D // H
        W = 256
        qkv = (lambda x, *d: x.transpose(*d))((x @ wqkv).reshape(B, S, 3, H, Dh), 2, 0, 3, 1, 4)
        q, k, v = (qkv[0], qkv[1], qkv[2])
        scores = jnp.einsum('bhqd,bhkd->bhqk', q, k) * Dh ** (-0.5)
        idx = jnp.arange(S)
        mask = (idx[:, None] - idx[None, :] >= 0) & (idx[:, None] - idx[None, :] < W)
        scores = jnp.where(mask[None, None], scores, -1000000000.0)
        p = _softmax(scores, axis=-1)
        o = jnp.einsum('bhqk,bhkd->bhqd', p, v)
        return (lambda x, *d: x.transpose(*d))(o, 0, 2, 1, 3).reshape(B, S, D) @ wo

    def _B_ref(x, mem0, Wq, Wk, Wv, Wo, seg_len):
        B, S, Dm = x.shape
        H, Dh = (Wq.shape[1], Wq.shape[2])
        M = mem0.shape[1]
        scale = Dh ** (-0.5)
        n_seg = S // seg_len
        L = M + seg_len
        idx = jnp.arange(L)
        mask = (idx[:, None] < M) | (idx[:, None] >= idx[None, :])
        mem = mem0
        outs = []
        for s in range(n_seg):
            xs = x[:, s * seg_len:(s + 1) * seg_len, :].copy()
            h = jnp.concatenate([mem, xs], axis=1)
            q = jnp.einsum('btd,dhe->bhte', h, Wq)
            k = jnp.einsum('btd,dhe->bhte', h, Wk)
            v = jnp.einsum('btd,dhe->bhte', h, Wv)
            scores = jnp.einsum('bhqe,bhke->bhqk', q, k) * scale
            scores = jnp.where(mask[None, None], scores, -1000000000.0)
            p = _softmax(scores, axis=-1)
            o = jnp.einsum('bhqk,bhke->bhqe', p, v)
            o = jnp.einsum('bhte,hed->btd', o, Wo)
            mem = o[:, :M, :].copy()
            outs.append(o[:, M:, :])
        return jnp.concatenate(outs, axis=1)
    x = A_x
    g = _sigmoid((x * gate_w).sum(-1, keepdims=True))
    a = _A_ref(x, A_wqkv, A_wo)
    b = _B_ref(x, B_mem0, B_Wq, B_Wk, B_Wv, B_Wo, B_seg_len)
    return g * a + (1 - g) * b
```

```python
import functools

import jax
import jax.numpy as jnp
from jax import lax
import jax.experimental.pallas as pl
import jax.experimental.pallas.tpu as pltpu

F32, BF16, U32, I32 = jnp.float32, jnp.bfloat16, jnp.uint32, jnp.int32
LOG2E = 1.4426950408889634
NEG = -1e9 * LOG2E

S, D = 2048, 448
DM = 384
HA, DA, WIN = 16, 28, 256
HB, DB, M = 16, 256, 8
SEG = 32
NP = HB // 2
BLK = 128
NB = S // BLK
TC = 512


def _dot(a, b):
    return lax.dot_general(a, b, (((1,), (0,)), ((), ())), preferred_element_type=F32)


def _dot_t(a, b):
    return lax.dot_general(a, b, (((1,), (1,)), ((), ())), preferred_element_type=F32)


def _pack(x):
    return pltpu.bitcast(x.astype(BF16), U32)


def _unpack(x):
    return pltpu.bitcast(x, BF16)


def _rnd(x):
    return x.astype(BF16).astype(F32)


def _cat0(xs):
    return jnp.concatenate(xs, axis=0)


def _cat1(xs):
    return jnp.concatenate(xs, axis=1)


def _iota(shape, dim):
    return lax.broadcasted_iota(I32, shape, dim)


def _allreduce8(x, op):
    lane = _iota(x.shape, 1)
    for s in (1, 2, 4):
        x = op(x, jnp.take_along_axis(x, lane ^ s, axis=1))
    return x


def _barrel(vs, n_out):
    grp = _iota(next(v for v in vs if v is not None).shape, 1) >> 4
    cur = {n: vs[(-n) % 8] for n in range(8)}

    def stage(n, bits):
        if not bits:
            return cur[n % 8]
        key = (n % 8, len(bits))
        if key not in memo:
            b = bits[0]
            lo, hi = stage(n, bits[1:]), stage(n - b, bits[1:])
            if lo is None or hi is None:
                zero = jnp.zeros(grp.shape, F32)
                if lo is None and hi is None:
                    memo[key] = None
                    return None
                lo = zero if lo is None else lo
                hi = zero if hi is None else hi
            memo[key] = jnp.where((grp & b) != 0, hi, lo)
        return memo[key]

    memo = {}
    return [stage(j, (1, 2, 4)) for j in range(n_out)]


def _roll(x, s):
    s %= 128
    return x if s == 0 else pltpu.roll(x, s, 1)


def _kernel(xT_hbm, wqkv_hbm, wo_hbm, mem_ref, wq_hbm, wk_hbm, wv_hbm, wob_hbm, gw_ref,
            out_hbm,
            xT_v, wqkv_v, wo_v, raw, wT_s, woT_s, wu_s, wt_s, wy_s, wz_s,
            xs_s, qT_s, vT_s, k_s, g_s, aT_s, b_s, o_s, out_v, in_sem, out_sem):
    c_wqkv = pltpu.make_async_copy(wqkv_hbm, wqkv_v, in_sem.at[0])
    c_x = [pltpu.make_async_copy(xT_hbm.at[:, pl.ds(t * TC, TC)], xT_v.at[t], in_sem.at[1 + t])
           for t in range(S // TC)]
    c_wo = pltpu.make_async_copy(wo_hbm, wo_v, in_sem.at[5])
    c_raw = [[pltpu.make_async_copy(w.bitcast(U32).at[:, pl.ds(128 * half, 128)], raw.at[2 * n + half],
                                    in_sem.at[6 + 2 * n + half]) for half in range(2)]
             for n, w in enumerate((wq_hbm, wk_hbm, wv_hbm, wob_hbm))]
    c_wqkv.start()
    for c in c_x:
        c.start()
    c_wo.start()
    for cs in c_raw:
        for c in cs:
            c.start()

    pad_lane = _iota((WIN, 128), 1) == 4 * DA
    for g in range(4):
        k_s[g, 0:WIN // 2, :] = _pack(jnp.where(pad_lane, NEG, 0.0))
    vT_s[0:2] = jnp.zeros((2, D, BLK), F32)
    aT_s[...] = jnp.zeros(aT_s.shape, F32)
    b_s[...] = jnp.zeros(b_s.shape, F32)

    c_wqkv.wait()
    wT_s[0:3 * D, :] = wqkv_v[...].astype(F32).T
    wT_s[3 * D:3 * D + 8, :] = jnp.broadcast_to(gw_ref[...].astype(F32).reshape(1, D), (8, D))

    def qkv_body(t, carry):
        pltpu.make_async_copy(xT_hbm.at[:, pl.ds(0, TC)], xT_v.at[t], in_sem.at[1 + t]).wait()
        xT = xT_v[t]
        r = _dot(wT_s[...], xT)
        xd = _cat0([xT, xT[DM:D]])
        row0 = pl.multiple_of(t * TC, TC)
        xs_s[pl.ds(row0, TC), :] = xd.T.astype(F32)
        for n in range(TC // BLK):
            blk = t * (TC // BLK) + n
            rn = r[:, n * BLK:(n + 1) * BLK]
            qT_s[blk] = rn[0:D] * (DA ** -0.5 * LOG2E)
            vT_s[blk + 2] = _rnd(rn[2 * D:3 * D])
            g_s[blk] = jax.nn.sigmoid(rn[3 * D:3 * D + 8])
        for g in range(4):
            kT = _cat0([r[D + 4 * DA * g:D + 4 * DA * (g + 1)], jnp.zeros((128 - 4 * DA, TC), F32)])
            k_s[g, pl.ds(pl.multiple_of(WIN // 2 + t * (TC // 2), 128), TC // 2), :] = (
                pltpu.bitcast(kT.astype(BF16).T, U32))
        return carry

    lax.fori_loop(0, S // TC, qkv_body, 0)

    c_wo.wait()
    woT_s[...] = wo_v[...].astype(F32).T

    def fold(la, lb, ra, rb):
        z = jnp.zeros((64, DB), BF16)
        fa = _dot_t(la, _cat0([ra, z]))
        fb = _dot_t(lb, _cat0([rb[0:DM], z, rb[DM:D]]))
        main = _cat1([fa[0:DM, 0:DM], fb[0:DM, 0:DM], fa[0:DM, DM:] + fb[0:DM, DM:]])
        return main, _cat0([fa[DM:D], fb[DM:D]])

    def head_pair(n, p):
        w = _cat1([raw[2 * n + half, pl.ds(p, D, stride=NP), :] for half in range(2)])
        return pltpu.bitcast(w << 16, F32), pltpu.bitcast(w & jnp.uint32(0xFFFF0000), F32)

    def qk_body(p, carry):
        qa, qb = head_pair(0, p)
        ka, kb = head_pair(1, p)
        main, tail = fold(ka, kb, qa.astype(BF16), qb.astype(BF16))
        sc = DB ** -0.5 * LOG2E
        wu_s[p] = _pack(main * sc)
        wt_s[p] = pltpu.bitcast((tail * sc).astype(BF16).T, U32)
        return carry

    def vo_body(p, carry):
        va, vb = head_pair(2, p)
        oa, ob = [_unpack(_cat1([raw[6 + half, pl.ds(pl.multiple_of((2 * p + e) * (D // 2), D // 2), D // 2), :]
                                 for half in range(2)])) for e in range(2)]
        main, tail = fold(va, vb, oa, ob)
        wy_s[p] = _pack(main)
        wz_s[p] = _pack(tail)
        return carry

    for c in c_raw[0] + c_raw[1]:
        c.wait()
    lax.fori_loop(0, NP, qk_body, 0)
    for c in c_raw[2] + c_raw[3]:
        c.wait()
    lax.fori_loop(0, NP, vo_body, 0)

    NJ = (M + SEG) // 8
    low = _iota((8, 128), 1) < 64

    def w_chunk(w_s, c):
        if c < 3:
            cols = [128 * c, DM + 128 * c]
        else:
            cols = [2 * DM]
        return _unpack(_cat1([w_s[p, :, o:o + 128] for p in range(NP) for o in cols]))

    def stack(u, c):
        rows = []
        for j in range(NJ):
            for p in range(NP):
                if c < 3:
                    rows += [u[8 * j:8 * j + 8, 256 * p:256 * p + 128], u[8 * j:8 * j + 8, 256 * p + 128:256 * p + 256]]
                else:
                    t = u[8 * j:8 * j + 8, 128 * p:128 * p + 128]
                    rows += [jnp.where(low, t, 0.0), jnp.where(low, 0.0, t)]
        return _cat0(rows).astype(BF16)

    tri = _iota((BLK, BLK), 0) > _iota((BLK, BLK), 1)

    def a_scores(i, h):
        g, j = divmod(h, 4)
        r0 = DA * j // 8 * 8
        q = qT_s[i, 4 * DA * g + r0:4 * DA * g + r0 + 32, :]
        row = _iota((32, BLK), 0) + r0
        q = jnp.where((row >= DA * j) & (row < DA * (j + 1)), q, 0.0)
        one = jnp.where(_iota((16, BLK), 0) == 0, 1.0, 0.0)
        parts = []
        if r0:
            parts.append(jnp.zeros((r0, BLK), F32))
        parts.append(q)
        if 4 * DA - r0 - 32:
            parts.append(jnp.zeros((4 * DA - r0 - 32, BLK), F32))
        parts.append(one)
        k = _unpack(k_s[g, pl.ds(pl.multiple_of(i * (BLK // 2), BLK // 2), 3 * BLK // 2), :])
        s = _dot(k, _cat0(parts).astype(BF16))
        s0 = jnp.where(tri, s[0:BLK], s[2 * BLK:])
        s1 = s[BLK:2 * BLK]
        m = jnp.max(jnp.maximum(s0, s1), axis=0, keepdims=True)
        p0 = jnp.exp2(s0 - m)
        p1 = jnp.exp2(s1 - m)
        l = jnp.sum(p0 + p1, axis=0, keepdims=True)
        p = _cat0([jnp.where(tri, p0, 0.0), p1, jnp.where(tri, 0.0, p0)]).astype(BF16)
        return p, l

    def a_values(i, h, pl_):
        p, l = pl_
        r0 = DA * h // 8 * 8
        v = _cat1([vT_s[i + n, r0:r0 + 32, :] for n in range(3)])
        return _dot(v, p) / l

    def mix(i):
        g = jnp.broadcast_to(g_s[i][0:1], (D, BLK))
        bT = b_s[...].T
        out_v[i] = (g * aT_s[...] + (1.0 - g) * bT[0:D]).astype(BF16)

    def out_copy(i):
        return pltpu.make_async_copy(out_v.at[i], out_hbm.at[:, pl.ds(pl.multiple_of(i * BLK, BLK), BLK)],
                                     out_sem.at[0])

    def step(mem, i, g, fill):
        x = xs_s[pl.ds(pl.multiple_of(i * BLK + g * SEG, SEG), SEG), :]
        h = _cat0([mem, x])
        hm = h[:, 0:DM]
        ht = []
        for j in range(NJ):
            t = h[8 * j:8 * j + 8, DM:]
            ht += [jnp.where(low, t, 0.0), jnp.where(low, 0.0, t)]
        ht = _cat0(ht + [jnp.zeros((128 - 16 * NJ, 128), F32)]).astype(BF16)

        t = _dot(h, _unpack(_cat1([wt_s[p] for p in range(NP)])))
        u0 = stack(_dot(hm, w_chunk(wu_s, 0)), 0).T
        st = _dot(_rnd(_cat0([t[:, 128 * p:128 * p + 128] for p in range(NP)])), ht.T)
        u1 = stack(_dot(hm, w_chunk(wu_s, 1)), 1).T
        u2 = stack(_dot(hm, w_chunk(wu_s, 2)), 2).T
        u3 = stack(_dot(hm, w_chunk(wu_s, 3)), 3).T
        y0 = stack(_dot(hm, w_chunk(wy_s, 0)), 0)
        s = _dot(h, _cat0([u0, u1, u2, u3]))
        y1 = stack(_dot(hm, w_chunk(wy_s, 1)), 1)

        causal = (_iota((8, 128), 1) & 7) <= _iota((8, 128), 0)
        ps, pz = [], []
        for qi in range(NJ):
            nj = NJ if qi == 0 else qi + 1
            rows = slice(8 * qi, 8 * qi + 8)
            tl = _barrel([_roll(st[40 * p + 8 * qi:40 * p + 8 * qi + 8], 16 * p) for p in range(NP)], nj)
            sj = [s[rows, 128 * j:128 * j + 128] + _roll(tl[j], -16 * j) for j in range(nj)]
            if qi:
                sj[qi] = jnp.where(causal, sj[qi], NEG)
            m = _allreduce8(functools.reduce(jnp.maximum, sj), jnp.maximum)
            e = [jnp.exp2(v - m) for v in sj]
            inv = 1.0 / _allreduce8(functools.reduce(jnp.add, e), jnp.add)
            pj = [_rnd(v * inv) for v in e]
            ps.append(_cat1(pj + [jnp.zeros((8, 128), F32)] * (NJ - nj)))
            pr = _barrel([_roll(v, 16 * j) for j, v in enumerate(pj)] + [None] * (8 - nj), NP)
            pz.append([_roll(pr[p], -16 * p) for p in range(NP)])
        pm = _cat0(ps)

        y2 = stack(_dot(hm, w_chunk(wy_s, 2)), 2)
        z = _dot(_cat0([pz[qi][p] for p in range(NP) for qi in range(NJ)]), ht)
        y3 = stack(_dot(hm, w_chunk(wy_s, 3)), 3)
        o = _dot(_rnd(_cat1([z[40 * p:40 * p + 40] for p in range(NP)])),
                 _unpack(_cat0([wz_s[p] for p in range(NP)])))
        fill(0)
        o = o + _dot(pm, _cat1([y0, y1, y2, y3]))
        fill(1)
        tail = o[:, DM:]
        b_s[g * SEG:(g + 1) * SEG, :] = _cat1([o[M:, 0:DM], tail[M:] + _roll(tail[M:], 64)])
        return _rnd(_cat1([o[0:M, 0:DM], tail[0:M] + _roll(tail[0:M], 64)]))

    heads = {(0, 0): (0, 1, 2), (0, 1): (3, 4, 5), (1, 0): (6, 7, 8), (1, 1): (9, 10), (2, 0): (11, 12, 13),
             (2, 1): (14, 15), (3, 0): (), (3, 1): ()}

    def body(i, mem):
        prev = jnp.maximum(i - 1, 0)
        mix(prev)
        pend, outs = [], {}

        def fill(g, n):
            done = list(pend)
            pend.clear()
            for h in heads[(g, n)]:
                pend.append((h, a_scores(i, h)))
            for h, p in done:
                outs[h] = a_values(i, h, p)
            if (g, n) == (3, 1):
                first = _iota((8, BLK), 0) < 4
                rows = []
                for h in range(0, HA, 2):
                    rows += [outs[h][0:24], jnp.where(first, outs[h][24:32], outs[h + 1][0:8]), outs[h + 1][8:32]]
                aT_s[...] = _dot(woT_s[...], _cat0(rows).astype(BF16))

        for g in range(4):
            mem = step(mem, i, g, functools.partial(fill, g))

        @pl.when(i > 0)
        def _():
            out_copy(prev).start()

        return mem

    mem0 = mem_ref[...].astype(F32)
    lax.fori_loop(0, NB, body, _cat1([mem0, mem0[:, DM:D]]))
    mix(NB - 1)
    out_copy(NB - 1).start()
    for i in range(NB):
        out_copy(i).wait()


@functools.partial(jax.jit, static_argnames=("B_seg_len",))
def pallas_gated_mix__sliding_block__memory_aug_recurrent_mem_tr__prompt_kernel(
    A_x, A_wqkv, A_wo, B_x, B_mem0, B_Wq, B_Wk, B_Wv, B_Wo, B_seg_len, gate_w,
):
    del B_x
    assert B_seg_len == SEG and A_x.shape == (1, S, D) and B_Wq.shape == (D, HB, DB) and B_mem0.shape == (1, M, D)
    hbm = pl.BlockSpec(memory_space=pl.ANY)
    vmem = pl.BlockSpec(memory_space=pltpu.VMEM)
    outT = pl.pallas_call(
        _kernel,
        out_shape=jax.ShapeDtypeStruct((D, S), BF16),
        in_specs=[hbm, hbm, hbm, vmem, hbm, hbm, hbm, hbm, vmem],
        out_specs=hbm,
        scratch_shapes=[
            pltpu.VMEM((S // TC, D, TC), BF16),
            pltpu.VMEM((D, 3 * D), BF16),
            pltpu.VMEM((D, D), BF16),
            pltpu.VMEM((8, D * NP, 128), U32),
            pltpu.VMEM((3 * D + 8, D), F32),
            pltpu.VMEM((D, D), F32),
            pltpu.VMEM((NP, DM // 2, 896), U32),
            pltpu.VMEM((NP, 256, 128), U32),
            pltpu.VMEM((NP, DM // 2, 896), U32),
            pltpu.VMEM((NP, 64, 512), U32),
            pltpu.VMEM((S, 512), F32),
            pltpu.VMEM((NB, D, BLK), F32),
            pltpu.VMEM((NB + 2, D, BLK), F32),
            pltpu.VMEM((4, (S + WIN) // 2, 128), U32),
            pltpu.VMEM((NB, 8, BLK), F32),
            pltpu.VMEM((D, BLK), F32),
            pltpu.VMEM((BLK, 512), F32),
            pltpu.VMEM((D // 2, BLK), U32),
            pltpu.VMEM((NB, D, BLK), BF16),
            pltpu.SemaphoreType.DMA((14,)),
            pltpu.SemaphoreType.DMA((1,)),
        ],
        compiler_params=pltpu.CompilerParams(vmem_limit_bytes=100 * 1024 * 1024),
    )(
        A_x[0].T, A_wqkv, A_wo, B_mem0[0],
        B_Wq.reshape(D * HB, DB), B_Wk.reshape(D * HB, DB), B_Wv.reshape(D * HB, DB),
        B_Wo.transpose(0, 2, 1).reshape(HB * D, DB), gate_w,
    )
    return outT.T[None]
```

```python
import functools

import jax
import jax.numpy as jnp
import numpy as np
from jax import lax
import jax.experimental.pallas as pl
import jax.experimental.pallas.tpu as pltpu

F32, BF16, U32, I32 = jnp.float32, jnp.bfloat16, jnp.uint32, jnp.int32
LOG2E = 1.4426950408889634
NEG = -1e9 * LOG2E

S, D = 2048, 448
DM, DT, HD = 384, 64, 224
DA, WIN = 28, 256
GA = 4 * DA
QG = 32
NK = WIN + QG
HB, DB, M, SEG = 16, 256, 8, 32
NP = HB // 2
NJ = (M + SEG) // 8
BLK = 128
NB = S // BLK
TC = 512

CLASSES = ((0, 0), (0, 4), (0, 1), (0, 3), (0, 2), (1, 0), (1, 1), (1, 2), (1, 3))

SCHEDULE = (
    "a.0 u.0.0.0 u.0.0.2 u.4.0.3 u.0.1.0 u.4.0.0 u.0.0.1 u.0.1.2 u.4.1.3 u.0.1.1 u.4.1.2 u.0.2.0 b.0 u.0.2.2 a.1 "
    "u.4.0.1 u.0.2.1 u.0.3.0 u.0.3.2 u.0.3.1 u.1.0.0 u.1.0.2 u.4.0.2 u.1.0.1 b.1 u.1.1.0 u.4.1.0 u.1.1.2 u.1.1.1 "
    "b.2 u.1.2.0 u.1.2.2 u.1.2.1 u.4.1.1 u.1.3.0 u.1.3.2 u.1.3.1 a.2 u.3.0.1 u.3.0.2 u.3.1.0 u.3.1.2 u.3.1.1 "
    "u.2.0.0 u.3.0.0 u.2.0.2 u.2.0.1 b.3 u.2.1.0 u.2.2.0 u.2.1.2 u.2.1.1 b.4 u.2.2.2 u.2.2.1 u.2.3.0 u.2.3.2 "
    "u.2.3.1 y.0.0.0 y.0.0.2 y.0.0.1 b.5 y.0.1.0 y.0.1.2 st.0 st.4 st.3 st.2 y.0.1.1 y.0.2.0 y.0.2.2 b.6 y.0.2.1 "
    "y.0.3.0 st.1 y.0.3.2 s.1 a.3 s.4 y.0.3.1 y.1.0.0 s.3 s.2 s.0 y.1.0.2 y.1.0.1 y.1.1.1 b.7 y.1.1.0 y.1.2.0 "
    "y.1.2.2 b.8 y.1.1.2 y.1.3.0 y.1.2.1 y.1.3.2 b.9 y.1.3.1 y.2.0.0 y.2.0.2 zt y.2.0.1 y.2.1.0 y.2.1.2 y.2.1.1 "
    "b.10 y.2.2.0 y.2.2.2 b.11 y.2.2.1 y.2.3.0 y.2.3.2 y.2.3.1 y.3.0.0 sm z.4.8 z.0.4 y.3.0.2 y.3.0.1 wz.1.0 "
    "y.3.1.0 wz.0.0 y.3.1.1 y.3.1.2 wz.1.1 wz.0.3 wz.0.1 wz.1.2 v.2 py.0 p wz.1.3 wz.0.2 py.1 py.2 py.3 py.4 v.1 "
    "v.3 v.0 ",
    "a.0 u.0.0.0 u.0.0.2 u.4.0.3 u.0.1.0 u.4.0.0 u.0.0.1 u.0.1.2 u.4.1.3 u.0.1.1 u.4.1.2 b.0 u.0.2.0 u.0.2.2 "
    "u.4.0.1 a.1 u.0.2.1 u.0.3.0 u.0.3.2 u.0.3.1 u.1.0.0 u.1.0.2 u.4.0.2 u.1.0.1 u.1.1.0 u.4.1.0 u.1.1.2 b.1 "
    "u.1.1.1 b.2 u.1.2.0 u.1.2.2 u.1.2.1 u.4.1.1 u.1.3.0 u.1.3.2 u.1.3.1 a.2 u.3.0.1 u.3.0.2 u.3.1.0 u.3.1.2 "
    "u.3.1.1 u.2.0.0 u.3.0.0 u.2.0.2 u.2.0.1 b.3 u.2.2.0 u.2.1.2 u.2.1.0 u.2.1.1 b.4 u.2.2.2 u.2.2.1 u.2.3.0 "
    "u.2.3.2 u.2.3.1 b.5 y.0.0.0 y.0.0.2 y.0.1.0 y.0.1.2 y.0.0.1 st.0 st.4 st.3 st.2 y.0.1.1 y.0.2.0 y.0.2.2 b.6 "
    "y.0.2.1 y.0.3.0 st.1 y.0.3.2 a.3 s.4 y.0.3.1 y.1.0.0 s.1 s.3 s.2 s.0 y.1.0.2 y.1.0.1 y.1.1.1 b.7 y.1.1.0 "
    "y.1.2.0 y.1.2.2 b.8 y.1.1.2 y.1.3.0 y.1.2.1 y.1.3.2 b.9 y.1.3.1 y.2.0.0 y.2.0.2 zt y.2.0.1 y.2.1.0 y.2.1.2 "
    "y.2.1.1 b.10 y.2.2.0 y.2.2.2 y.2.2.1 y.2.3.0 sm z.4.8 b.11 y.2.3.2 y.2.3.1 y.3.0.0 z.0.4 y.3.0.2 y.3.0.1 "
    "wz.1.0 y.3.1.0 wz.0.0 y.3.1.1 wz.0.3 y.3.1.2 wz.1.1 wz.0.1 wz.1.2 v.2 py.0 p wz.1.3 wz.0.2 py.1 py.2 py.3 "
    "py.4 v.1 v.3 v.0 ",
    "a.0 u.0.0.0 u.0.0.2 u.4.0.3 u.0.1.0 u.4.0.0 u.0.0.1 u.0.1.2 u.4.1.3 u.0.1.1 u.4.1.2 u.0.2.0 b.0 u.0.2.2 "
    "u.4.0.1 a.1 u.0.2.1 u.0.3.0 u.0.3.2 u.0.3.1 u.1.0.0 u.1.0.2 u.4.0.2 u.1.0.1 b.1 u.1.1.0 u.4.1.0 u.1.1.2 "
    "u.1.3.0 u.1.1.1 b.2 u.1.2.0 u.1.2.2 u.1.2.1 u.4.1.1 u.1.3.2 u.1.3.1 a.2 u.3.0.1 u.3.0.2 u.3.1.0 u.3.1.2 "
    "u.3.1.1 u.2.0.0 u.3.0.0 u.2.0.2 u.2.0.1 b.3 u.2.1.0 u.2.2.0 u.2.1.2 u.2.1.1 b.4 u.2.2.2 u.2.2.1 u.2.3.0 "
    "u.2.3.2 u.2.3.1 y.0.0.0 b.5 y.0.0.2 y.0.0.1 y.0.1.0 y.0.1.2 st.0 st.4 st.3 st.2 y.0.1.1 y.0.2.0 y.0.2.2 b.6 "
    "y.0.2.1 y.0.3.0 st.1 y.0.3.2 a.3 y.0.3.1 y.1.0.0 s.3 s.1 s.2 s.0 s.4 y.1.0.2 y.1.0.1 y.1.1.1 b.7 y.1.1.0 "
    "y.1.2.0 y.1.2.2 y.1.1.2 y.1.3.0 b.8 y.1.2.1 y.1.3.2 y.1.3.1 y.2.0.0 b.9 y.2.0.2 zt y.2.0.1 y.2.1.0 y.2.1.2 "
    "y.2.1.1 b.10 y.2.2.0 y.2.2.2 y.2.2.1 b.11 y.2.3.0 sm z.4.8 y.2.3.2 y.2.3.1 y.3.0.0 z.0.4 y.3.0.2 y.3.0.1 "
    "wz.1.0 y.3.1.0 wz.0.0 y.3.1.1 y.3.1.2 wz.1.1 wz.1.2 wz.0.3 v.2 wz.0.1 py.0 p wz.1.3 wz.0.2 py.1 py.2 py.3 "
    "py.4 v.3 v.0 v.1 ",
    "a.0 u.0.0.0 u.0.0.2 u.4.0.3 u.0.1.0 u.4.0.0 u.0.0.1 u.0.1.2 u.4.1.3 u.0.1.1 u.4.1.2 u.0.2.0 b.0 u.0.2.2 "
    "u.4.0.1 u.0.2.1 u.0.3.0 u.0.3.2 a.1 u.0.3.1 u.1.0.0 u.1.0.2 u.1.0.1 u.1.1.0 u.4.1.0 u.1.1.2 u.4.0.2 b.1 "
    "u.1.1.1 b.2 u.1.2.0 u.1.2.2 u.1.2.1 u.4.1.1 u.1.3.0 u.1.3.2 u.1.3.1 a.2 u.3.0.1 u.3.0.2 u.3.1.0 u.3.1.2 "
    "u.3.1.1 u.2.0.0 u.3.0.0 u.2.0.2 u.2.0.1 b.3 u.2.1.0 u.2.2.0 u.2.1.2 u.2.1.1 b.4 u.2.2.2 u.2.2.1 u.2.3.0 "
    "u.2.3.2 u.2.3.1 b.5 y.0.0.0 y.0.0.2 y.0.1.0 y.0.1.2 y.0.0.1 st.0 st.4 st.3 st.2 y.0.1.1 y.0.2.0 y.0.2.2 b.6 "
    "y.0.2.1 y.0.3.0 st.1 y.0.3.2 a.3 s.4 s.1 y.0.3.1 y.1.0.0 s.3 s.2 s.0 y.1.0.2 y.1.0.1 y.1.1.1 b.7 y.1.1.0 "
    "y.1.2.0 y.1.2.2 y.1.1.2 y.1.3.0 y.1.2.1 b.8 y.1.3.2 b.9 y.1.3.1 y.2.0.0 y.2.0.2 zt y.2.0.1 y.2.1.0 y.2.1.2 "
    "y.2.1.1 b.10 y.2.2.0 y.2.2.2 y.2.2.1 y.2.3.0 sm z.4.8 b.11 y.3.0.0 y.2.3.2 y.2.3.1 z.0.4 y.3.0.2 y.3.0.1 "
    "wz.1.0 y.3.1.0 wz.0.0 y.3.1.1 y.3.1.2 wz.1.1 wz.0.3 wz.1.2 v.2 wz.0.1 py.0 p wz.1.3 wz.0.2 py.2 py.1 py.3 "
    "py.4 v.1 v.3 v.0 ",
)


def _dot(a, b):
    return lax.dot_general(a, b, (((1,), (0,)), ((), ())), preferred_element_type=F32)


def _dot_t(a, b):
    return lax.dot_general(a, b, (((1,), (1,)), ((), ())), preferred_element_type=F32)


def _pack(x):
    return pltpu.bitcast(x, U32)


def _unpack(x):
    return pltpu.bitcast(x, BF16)


def _put(dst, x, tile=0):
    dst[:, 128 * tile:128 * tile + x.shape[1]] = _pack(x.astype(BF16))


def _rnd(x):
    return x.astype(BF16).astype(F32)


def _cat0(xs):
    return jnp.concatenate(xs, axis=0)


def _cat1(xs):
    return jnp.concatenate(xs, axis=1)


def _tile(n, width=128):
    return slice(width * n, width * (n + 1))


def _iota(shape, dim):
    return lax.broadcasted_iota(I32, shape, dim)


def _roll(x, s):
    return pltpu.roll(x, s, 1) if s else x


def _add_rows(x, y):
    if x.shape[0] < y.shape[0]:
        x, y = y, x
    n = y.shape[0]
    return x + y if n == x.shape[0] else _cat0([x[0:n] + y, x[n:]])


def _allreduce8(x, op):
    lane = _iota(x.shape, 1)
    return functools.reduce(op, [jnp.take_along_axis(x, lane ^ s, axis=1) for s in range(1, 8)], x)


def _transpose8(x):
    row, lane = _iota(x.shape, 0), _iota(x.shape, 1)
    x = jnp.take_along_axis(x, (lane & ~7) | ((row - lane) & 7), axis=1)
    for b in (1, 2, 4):
        x = jnp.where((lane & b) != 0, pltpu.roll(x, 8 - b, 0), x)
    return jnp.take_along_axis(x, (lane & ~7) | ((lane - row) & 7), axis=1)


def _barrel(vs):
    grp = _iota((8, 128), 1) >> 4
    zero = jnp.zeros((8, 128), F32)

    @functools.cache
    def stage(n, bit):
        if bit == 8:
            return vs[-n % 8] if -n % 8 < len(vs) else None
        lo, hi = stage(n, 2 * bit), stage((n - bit) % 8, 2 * bit)
        if lo is None and hi is None:
            return None
        return jnp.where((grp & bit) != 0, zero if hi is None else hi, zero if lo is None else lo)

    return [stage(p, 1) for p in range(8)]


def _strassen_weights(left, right):
    b11, b12, b21, b22 = left[0], right[0], left[1], right[1]
    ws = [b11 + b22, b12 - b22, b22, b21 + b22, b11, b21 - b11, b11 + b12]
    for l, r in zip(left[2:], right[2:]):
        ws += [l, r]
    return ws


def _phase(cls, b):
    return (CLASSES.index(cls) + b) % 4


def _kernel(xT_hbm, wqkv_hbm, wo_hbm, mem_hbm, wq_hbm, wk_hbm, wv_hbm, wob_hbm, gw_hbm,
            out_hbm,
            xT_v, wqkv_v, wo_v, mem_v, gw_v, gw_s, raw, wT_s, woT_s, w_s, wz_s, wzT_s, z_s, zT_s, ahead_s, lhs_s,
            xs_s, xb_s, qT_s, qm_s, vT_s, k_s, g_s, o_s, b_s, bT_s, y_s, ht_s, p_s, out_v, in_sem, out_sem):
    sems = iter(range(S // TC, in_sem.shape[0]))

    def copy(src, dst):
        c = pltpu.make_async_copy(src, dst, in_sem.at[next(sems)])
        c.start()
        return c

    def x_copy(t):
        return pltpu.make_async_copy(xT_hbm.at[:, pl.ds(t * TC, TC)], xT_v.at[t], in_sem.at[t])

    def w_copy(c0, c1):
        return copy(wqkv_hbm.at[:, pl.ds(c0, c1 - c0)], wqkv_v.at[:, pl.ds(c0, c1 - c0)])

    c_w0 = w_copy(0, 512)
    x_copy(0).start()
    c_w1 = w_copy(512, 3 * D)
    c_gw = copy(gw_hbm, gw_v)

    pad = _pack(jnp.where(_iota((WIN, 128), 1) >= GA, NEG, 0.0).astype(BF16))
    for g in range(4):
        k_s[g, 0:WIN // 2, :] = pad
    vT_s[0:2] = jnp.zeros((2, D, BLK), F32)
    row, col = _iota((64, 4 * BLK), 0), _iota((64, 4 * BLK), 1)
    slot = ((col >> 5) - (col >> 7)) & 3
    keep = (row >= slot * (DA // 2)) & (row < (slot + 1) * (DA // 2))
    one = jnp.where((slot & 1) == 0, np.uint32(0x00003F80), np.uint32(0x3F800000))
    qm_s[...] = jnp.where(keep, np.uint32(0xFFFFFFFF), jnp.where(row == GA // 2 + (slot >> 1), one, np.uint32(0)))
    o_s[...] = jnp.zeros(o_s.shape, U32)
    z_s[...] = jnp.zeros(z_s.shape, U32)
    b_s[...] = jnp.zeros(b_s.shape, F32)

    def transpose_w(c0, c1):
        for e in range(2):
            w = _cat0([wqkv_v[_tile(e, HD), c0:c1], jnp.zeros((256 - HD, c1 - c0), BF16)])
            wT_s[e, c0 // 2:c1 // 2, :] = _pack(w.T)

    def qkv_chunk(t):
        xT = xT_v[t]
        xf = xT.astype(F32)
        b11, b12, b21, b22 = [xf[_tile(e, HD), _tile(f, TC // 2)] for e in range(2) for f in range(2)]
        rhs = [_cat0([r, jnp.zeros((256 - HD, TC // 2), F32)]).astype(BF16)
               for r in (b11 + b22, b11, b12 - b22, b21 - b11, b22, b11 + b12, b21 + b22)]

        def project_rows(n):
            a11, a12, a21, a22 = [_unpack(wT_s[e, _tile(r, HD // 2), :]).astype(F32)
                                  for r in (2 * n, 2 * n + 1) for e in range(2)]
            m1, m2, m3, m4, m5 = [_dot(l, r) for l, r in zip((a11 + a22, a21 + a22, a11, a22, a11 + a12), rhs)]
            if t == 0 and n == 0:
                c_w1.wait()
                c_gw.wait()
                transpose_w(512, 3 * D)
                gw_s[...] = jnp.broadcast_to(gw_v[...].astype(F32).reshape(1, D), (BLK, D)).T
            m6, m7 = _dot(a21 - a11, rhs[5]), _dot(a12 - a22, rhs[6])
            return _cat0([_cat1([m1 + m4 - m5 + m7, m3 + m5]), _cat1([m2 + m4, m1 - m2 + m3 + m6])])

        blk = t * (TC // BLK)
        q = project_rows(0)
        for n in range(TC // BLK):
            _put(qT_s.at[blk + n], _cat1([q[_tile(g, GA), _tile(n)] for g in range(4)]) * (DA ** -0.5 * LOG2E))
        xs_s[_tile(t, TC), :] = _cat0([xT, xT[DM:D]]).T.astype(F32)
        k = project_rows(1)
        for g in range(4):
            kT = _cat0([k[_tile(g, GA)], jnp.zeros((128 - GA, TC), F32)])
            k_s[g, (WIN + t * TC) // 2:(WIN + (t + 1) * TC) // 2, :] = _pack(kT.astype(BF16).T)
        v = project_rows(2)
        for n in range(TC // BLK):
            vT_s[blk + n + 2] = v[:, _tile(n)]
            logit = jnp.sum(xf[:, _tile(n)] * gw_s[...], axis=0, keepdims=True)
            g_s[blk + n] = jax.nn.sigmoid(jnp.broadcast_to(logit, (8, BLK)))

    c_w0.wait()
    for t in range(1, S // TC):
        x_copy(t).start()
    c_wo = copy(wo_hbm, wo_v)
    c_mem = copy(mem_hbm, mem_v.at[0])
    c_raw = [[copy(w.bitcast(U32).at[:, pl.ds(128 * e, 128)], raw.at[2 * m + e, pl.ds(0, D * NP)])
              for e in range(2)] for m, w in enumerate((wq_hbm, wk_hbm, wv_hbm, wob_hbm))]
    transpose_w(0, 512)
    x_copy(0).wait()
    qkv_chunk(0)
    for t in range(1, S // TC):
        x_copy(t).wait()
    for t in range(1, S // TC):
        qkv_chunk(t)

    def head_pair(n, p):
        w = _cat1([raw[2 * n + e, pl.ds(p, D, stride=NP), :] for e in range(2)])
        return pltpu.bitcast(w << 16, F32), pltpu.bitcast(w & np.uint32(0xFFFF0000), F32)

    def fold(la, lb, ra, rb):
        la, lb = _cat0([la[DM:D], la[0:DM]]), _cat0([lb[DM:D], lb[0:DM]])
        fa = _dot_t(la, ra[0:256].astype(BF16))
        ta = _dot_t(ra[DM:D], la.astype(BF16))
        fa = _cat1([fa, _dot_t(la, ra[256:DM].astype(BF16))])
        fb = _dot_t(lb, rb[0:128].astype(BF16))
        tb = _dot_t(rb[DM:D], lb.astype(BF16))
        tl = _cat0([ta, tb]).astype(BF16).T.astype(F32)
        fb = _cat1([fb, _dot_t(lb, rb[128:DM].astype(BF16))])
        lo = _iota((DT, 128), 1) < DT
        main = _cat1([fa[DT:], fb[DT:], tl[DT:]])
        tail = _cat0([_cat1([fa[0:DT], jnp.where(lo, tl[0:DT], 0.0)]), _cat1([fb[0:DT], jnp.where(lo, 0.0, tl[0:DT])])])
        return main, tail, jnp.where(lo, ta[:, 0:128], _roll(tb[:, 0:128], DT))

    def store_folded(side, n, mains):
        def tiles(x, col):
            return [x[_tile(k), col:col + 128] for k in range(3)]

        for c in range(3):
            ws = [_strassen_weights(tiles(m, 128 * c), tiles(m, DM + 128 * c)) for m in mains]
            for m in range(9):
                _put(w_s.at[side, n, c, m], _cat1([ws[0][m], ws[1][m]]))
        for m, w in enumerate(_strassen_weights(tiles(mains[0], 2 * DM), tiles(mains[1], 2 * DM))):
            _put(w_s.at[side, n, 3, m], w)
        for s, c in sorted(CLASSES):
            if s == side:
                cols = slice(0, 256) if c < 3 else _tile(c - 3)
                for b in range(3):
                    rows = slice(0, 16 * (_phase((s, c), b) + 1))
                    ahead_s[s, n, min(c, 3), b, rows, cols] = _dot(
                        lhs_s[b, rows, :], _unpack(w_s[s, n, min(c, 3), 4 + b, :, cols]))

    def ahead_lhs(x, g):
        a11, a21, a22 = x[0:16, 0:128], x[16:32, 0:128], x[16:32, 128:256]
        for b, l in enumerate((a21 + a22, a22, a21 - a11)):
            lhs_s[b, _tile(g, 16), :] = l

    def fold_scores(n):
        mains, tails = [], []
        for e in range(2):
            qa, qb = head_pair(0, 2 * n + e)
            ka, kb = head_pair(1, 2 * n + e)
            main, tail, _ = fold(ka, kb, qa, qb)
            mains.append(main)
            tails.append([tail[:, _tile(k)] for k in range(4)])
            if e == 0:
                w = wo_v[_tile(n, GA), :]
                woT_s[n] = _pack(_cat0([w, jnp.zeros((128 - GA, D), BF16)]).T)
        for m, w in enumerate(_strassen_weights(*tails)):
            w_s[0, n, 3, m, :, 128:256] = _pack(w.astype(BF16).T)
        store_folded(0, n, mains)

    def fold_outputs(n):
        mains = []
        for e in range(2):
            p = 2 * n + e
            va, vb = head_pair(2, p)
            oa, ob = [_unpack(_cat1([raw[6 + half, pl.ds(pl.multiple_of((2 * p + f) * HD, HD), HD), :]
                                     for half in range(2)])) for f in range(2)]
            main, tail, corner = fold(va, vb, oa, ob)
            mains.append(main)
            _put(wz_s.at[p], tail)
            wzT_s[p] = corner
        store_folded(1, n, mains)

    c_wo.wait()
    for g in range(4):
        ahead_lhs(xs_s[_tile(g, SEG), 0:256], g)
    for c in c_raw[0] + c_raw[1]:
        c.wait()
    for n in range(NP // 2):
        fold_scores(n)
    for c in c_raw[2] + c_raw[3]:
        c.wait()

    @pl.loop(0, NP // 4)
    def _(n):
        fold_outputs(2 * n)
        fold_outputs(2 * n + 1)

    def a_keys(i, g):
        k = k_s[g, pl.ds(pl.multiple_of(i * (BLK // 2), BLK // 2), 3 * BLK // 2), :]
        lane = _iota((8, 128), 1)
        slot = jnp.where(lane >= GA, lane - GA, sum((lane >= DA * j).astype(I32) for j in (1, 2, 3)))

        def shift(bit, off, x, n):
            return _cat0([jnp.where(bit, x[off + r:off + r + 8], x[r:r + 8]) for r in range(0, n, 8)])

        half = [shift(((slot + v) & 1) != 0, QG // 2, k, (NK + 2 * QG) // 2) for v in range(2)]
        return [shift(((slot + v) & 2) != 0, QG, half[v % 2], NK // 2) for v in range(4)]

    def a_scores(i, g, v, k):
        q = _cat0([qT_s[i, :, _tile(g)] & qm_s[0:GA // 2, _tile(v)], qm_s[GA // 2:64, _tile(v)]])
        k = _unpack(k).astype(F32)
        s = _cat0([_dot(k[_tile(n, NK // 4)], _unpack(q)) for n in range(4)])
        oldest = _iota((QG, BLK), 0) > (_iota((QG, BLK), 1) & (QG - 1))
        s = _cat0([jnp.where(oldest, s[0:QG], s[WIN:NK]), s[QG:WIN]])
        p = jnp.exp2(s - jnp.max(s, axis=0, keepdims=True))
        _put(p_s, _cat0([jnp.where(oldest, p[0:QG], 0.0), p[QG:WIN], jnp.where(oldest, 0.0, p[0:QG])]), v)
        return p_s[:, _tile(v)]

    def a_values(i, g, probs):
        lane = _iota((8, 128), 1)
        zero = jnp.zeros((8, 128), U32)

        def unshift(bit, off, lo, hi):
            n = lo.shape[0]
            return _cat0([jnp.where(bit, hi[r - off:r - off + 8] if r >= off else zero, lo[r:r + 8] if r < n else zero)
                          for r in range(0, n + off, 8)])

        b0, b1 = (lane & QG) != 0, (lane & (2 * QG)) != 0
        half = [unshift(b0, QG // 2, probs[v], probs[(v + 1) % 4]) for v in range(4)]

        def head(j):
            p = _unpack(unshift(b1, QG, half[-j % 4], half[(2 - j) % 4]))
            r0 = DA * (4 * g + j) // 8 * 8
            vT = _cat1([vT_s[i + n, r0:r0 + 32, :] for n in range(3)])
            first = _iota((8, 3 * BLK), 0) < 4
            if j % 2:
                o = _dot(_cat0([jnp.where(first, 1.0, vT[0:8]), vT[8:]]), p)
                return o * (1.0 / o[0:1])
            o = _dot(_cat0([vT[0:24], jnp.where(first, vT[24:], 1.0)]), p)
            return o * (1.0 / o[31:32])

        return head

    def a_merge(outs):
        first = _iota((8, BLK), 0) < 4
        rows = []
        for j in (0, 2):
            rows += [outs[j][0:24], jnp.where(first, outs[j][24:32], outs[j + 1][0:8]), outs[j + 1][8:32]]
        return _cat0(rows + [jnp.zeros((128 - GA, BLK), F32)])

    def latch_block():
        bT_s[...] = b_s[...].T
        o_s[1] = o_s[0]
        zT_s[...] = _pack(_unpack(_cat0([z_s[g] for g in range(4)])).T)

    def token_corner(half):
        bT_s[DM:D, :] += _dot(_cat1([wzT_s[p] for p in range(4 * half, 4 * half + 4)]),
                              _unpack(zT_s[_tile(half, 256), :]))

    def mix(i, n):
        a = _dot(_unpack(_cat1([woT_s[m, _tile(n, GA // 2), :] for m in range(4)])),
                 _unpack(_cat0([o_s[1, :, _tile(m)] for m in range(4)])))
        g = jnp.broadcast_to(g_s[i][0:1], a.shape)
        out_v[i, _tile(n, GA), :] = (g * a + (1.0 - g) * bT_s[_tile(n, GA), :]).astype(BF16)

    def out_copy(i):
        return pltpu.make_async_copy(out_v.at[i], out_hbm.at[:, pl.ds(pl.multiple_of(i * BLK, BLK), BLK)],
                                     out_sem.at[0])

    low = _iota((8, 128), 1) < DT

    def columns(side, c, q, m, rows=slice(None)):
        if c < 3:
            return [(side, q, c, m, rows, slice(0, 256))]
        return [(side, n, 3, m, rows, _tile(c - 3)) for n in (2 * q, 2 * q + 1)]

    def stack(groups, c):
        out = []
        for j in range(NJ):
            rows = []
            for left, right in groups:
                for k in range(2):
                    a, b = left[_tile(j, 8), _tile(k)], right[_tile(j, 8), _tile(k)]
                    if c < 3:
                        rows += [a, b]
                    else:
                        rows += [jnp.where(low, a, 0.0), jnp.where(low, 0.0, a),
                                 jnp.where(low, b, 0.0), jnp.where(low, 0.0, b)]
            out.append(_cat0(rows))
        return out

    def step(mem, i, g):
        x = xb_s[_tile(g, SEG), :]
        h = _cat0([mem, x])
        for j in range(NJ):
            t = h[_tile(j, 8), DM:]
            _put(ht_s, _cat0([jnp.where(low, t, 0.0), jnp.where(low, 0.0, t)]), j)
        nxt = jnp.minimum(i + 1, NB - 1)
        x_next = xs_s[pl.ds(pl.multiple_of(nxt * BLK + g * SEG, SEG), SEG), :]
        ahead_lhs(x_next, g)
        a11, a12, a22 = h[0:24, 0:128], h[0:24, 128:256], x[16:32, 128:256]
        lhs = [_cat0([a11[0:M], a11[M:] + a22]), a11, a11 + a12, _cat0([a12[0:M], a12[M:] - a22])]
        v, stale = {}, []

        def project(side, c, q, part):
            def w(m):
                return _cat1([w_s[idx] for idx in columns(side, c, q, m)])

            if part < 2:
                r = [_dot(lhs[m], _unpack(w(m))) for m in (2 * part, 2 * part + 1)]
            else:
                r = _dot(h[:, _tile(part)], _unpack(_cat1([w(2 * part + 3), w(2 * part + 4)])))
                r = [r[:, 0:256], r[:, 256:512]]
            if part == 0:
                m2, m4, m6 = [_cat1([ahead_s[idx] for idx in columns(side, c, q, b, _tile(g, 16))]) for b in range(3)]
                m1, m3 = r
                r = [_cat0([m1[0:M], m1[M:] + m4, m2 + m4]), _cat0([m3, m1[M:] + m3[M:] + (m6 - m2)])]
            elif part == 1:
                r = [r[1] - r[0], r[0]]
            if ("sum", side, c, q) in v:
                r = [_add_rows(acc, new) for acc, new in zip(v["sum", side, c, q], r)]
            v["sum", side, c, q] = r
            v["left", side, c, q] = v.get(("left", side, c, q), 4 if c == 4 else 3) - 1
            if v["left", side, c, q]:
                return
            if v.get(("left", side, c, q ^ 1)) == 0:
                stale.extend((side, c, q & ~1, b) for b in range(3) if _phase((side, c), b) == g)
            qs = range(4 if c < 3 else 2)
            if all(v.get(("left", side, c, k)) == 0 for k in qs):
                tiles = stack([v["sum", side, c, k] for k in qs], c)
                if side:
                    _put(y_s.at[c], _cat1(tiles))
                else:
                    v["u", c] = _pack(_cat0(tiles).astype(BF16).T)

        def refresh(*_):
            if stale:
                side, c, q, b = stale.pop(0)
                r = _dot(lhs_s[b], _unpack(_cat1([w_s[idx] for k in (q, q + 1) for idx in columns(side, c, k, 4 + b)])))
                idxs = columns(side, c, q, b) + columns(side, c, q + 1, b)
                for n, idx in enumerate(idxs):
                    ahead_s[idx] = r[:, _tile(n, 512 // len(idxs))]

        def n_keys(qi):
            return qi + 1 if qi else NJ

        def tail_scores(qi):
            v["st", qi] = _dot(h[0:8 * n_keys(qi), DM:], _unpack(v["u", 4][:, _tile(qi)]))

        def scores(j):
            qs = [qi for qi in range(NJ) if j < n_keys(qi)]
            s = _dot(_cat0([h[_tile(qi, 8)] for qi in qs]), _unpack(_cat0([v["u", c][:, _tile(j)] for c in range(4)])))
            for n, qi in enumerate(qs):
                v["s", qi, j] = s[_tile(n, 8)]

        def softmax():
            causal = (_iota((8, 128), 1) & 7) <= _iota((8, 128), 0)
            for qi in range(NJ):
                s = [(v["s", qi, j] + _transpose8(v["st", qi][_tile(j, 8)])) * (DB ** -0.5 * LOG2E)
                     for j in range(n_keys(qi))]
                if qi:
                    s[qi] = jnp.where(causal, s[qi], NEG)
                m = _allreduce8(functools.reduce(jnp.maximum, s), jnp.maximum)
                e = [jnp.exp2(t - m) for t in s]
                inv = 1.0 / _allreduce8(functools.reduce(jnp.add, e), jnp.add)
                v["p", qi] = [_rnd(t * inv) for t in e]
                v["pz", qi] = _barrel([_roll(t, 16 * j) for j, t in enumerate(v["p", qi])])

        def tail_values(p0, p1):
            zero = jnp.zeros((8, 128), U32)
            for p in range(p0, p1):
                ht = _cat0([ht_s[:, _tile((n - p) % 8)] if (n - p) % 8 < NJ else zero for n in range(8)])
                v["z", p] = _dot(_cat0([v["pz", qi][p] for qi in range(NJ)]), _unpack(ht))

        def add_out(qs, c, o):
            for n, qi in enumerate(qs):
                v["o", qi, c] = v["o", qi, c] + o[_tile(n, 8)] if ("o", qi, c) in v else o[_tile(n, 8)]

        def tail_out(half, c):
            ps = range(4 * half, 4 * half + 4)
            z = _cat1([v["z", p] for p in ps])
            if c == 3:
                _put(z_s.at[g], z[M:], 4 * half)
                z = z[0:M]
            add_out(range(z.shape[0] // 8), c, _dot(z, _unpack(_cat0([wz_s[p, :, _tile(c)] for p in ps]))))

        def values(j):
            qs = [qi for qi in range(NJ) if j < n_keys(qi)]
            o = _dot(_cat0([v["p", qi][j] for qi in qs]), _unpack(_cat1([y_s[c, :, _tile(j)] for c in range(4)])))
            for c in range(4):
                add_out(qs, c, o[:, _tile(c)])

        def window_scores(n):
            if "k" not in v:
                v["k"] = a_keys(i, g)
            v["a", n] = a_scores(i, g, n, v["k"][n])

        def window_values(j):
            if "head" not in v:
                v["head"] = a_values(i, g, [v["a", n] for n in range(4)])
            v["av", j] = v["head"](j)
            if all(("av", n) in v for n in range(4)):
                _put(o_s.at[0], a_merge([v["av", n] for n in range(4)]), g)

        ops = dict(u=functools.partial(project, 0), y=functools.partial(project, 1), b=refresh,
                   st=tail_scores, s=scores, sm=softmax, z=tail_values, wz=tail_out, py=values,
                   a=window_scores, v=window_values,
                   zt=lambda: token_corner(g) if g < 2 else None, p=lambda: mix(jnp.maximum(i - 1, 0), g))
        for item in SCHEDULE[g].split():
            name, *args = item.split(".")
            ops[name](*map(int, args))
        while stale:
            refresh()
        xb_s[_tile(g, SEG), :] = x_next
        o = _cat0([_cat1([v["o", qi, c] for c in range(4)]) for qi in range(NJ)])
        tail = o[:, DM:]
        b_s[_tile(g, SEG), :] = _cat1([o[M:, 0:DM], tail[M:] + _roll(tail[M:], DT)])
        return _rnd(_cat1([o[0:M, 0:DM], tail[0:M] + _roll(tail[0:M], DT)]))

    def body(i, mem):
        latch_block()
        for g in range(4):
            mem = step(mem, i, g)

        @pl.when(i > 0)
        def _():
            out_copy(i - 1).start()

        return mem

    c_mem.wait()
    xb_s[...] = xs_s[0:BLK, :]
    mem0 = mem_v[0].astype(F32)
    lax.fori_loop(0, NB, body, _cat1([mem0, mem0[:, DM:D]]))
    latch_block()
    for n in range(4):
        if n >= 2:
            token_corner(n - 2)
        mix(NB - 1, n)
    out_copy(NB - 1).start()
    for i in range(NB):
        out_copy(i).wait()


@functools.partial(jax.jit, static_argnames=("B_seg_len",))
def pallas_gated_mix__sliding_block__memory_aug_recurrent_mem_tr__prompt_kernel(
    A_x, A_wqkv, A_wo, B_x, B_mem0, B_Wq, B_Wk, B_Wv, B_Wo, B_seg_len, gate_w,
):
    del B_x
    assert B_seg_len == SEG and A_x.shape == (1, S, D) and B_Wq.shape == (D, HB, DB) and B_mem0.shape == (1, M, D)
    hbm = pl.BlockSpec(memory_space=pl.ANY)
    outT = pl.pallas_call(
        _kernel,
        out_shape=jax.ShapeDtypeStruct((D, S), BF16),
        in_specs=[hbm] * 9,
        out_specs=hbm,
        scratch_shapes=[
            pltpu.VMEM((S // TC, D, TC), BF16),
            pltpu.VMEM((D, 3 * D), BF16),
            pltpu.VMEM((D, D), BF16),
            pltpu.VMEM((2, M, D), BF16),
            pltpu.VMEM((D,), BF16),
            pltpu.VMEM((D, BLK), F32),
            pltpu.VMEM((8, D * NP + 8, 128), U32),
            pltpu.VMEM((2, 3 * HD, 256), U32),
            pltpu.VMEM((4, HD, 128), U32),
            pltpu.VMEM((2, NP // 2, 4, 11, 64, 256), U32),
            pltpu.VMEM((NP, 64, 512), U32),
            pltpu.VMEM((NP, DT, 128), F32),
            pltpu.VMEM((4, SEG // 2, 1024), U32),
            pltpu.VMEM((512, BLK), U32),
            pltpu.VMEM((2, NP // 2, 4, 3, 64, 256), F32),
            pltpu.VMEM((3, 64, 128), F32),
            pltpu.VMEM((S, 512), F32),
            pltpu.VMEM((BLK, 512), F32),
            pltpu.VMEM((NB, GA // 2, 4 * BLK), U32),
            pltpu.VMEM((64, 4 * BLK), U32),
            pltpu.VMEM((NB + 2, D, BLK), F32),
            pltpu.VMEM((4, (S + WIN) // 2, 128), U32),
            pltpu.VMEM((NB, 8, BLK), F32),
            pltpu.VMEM((2, 64, 4 * BLK), U32),
            pltpu.VMEM((BLK, 512), F32),
            pltpu.VMEM((512, BLK), F32),
            pltpu.VMEM((4, 64, 640), U32),
            pltpu.VMEM((8, 640), U32),
            pltpu.VMEM((NK // 2, 512), U32),
            pltpu.VMEM((NB, D, BLK), BF16),
            pltpu.SemaphoreType.DMA((17,)),
            pltpu.SemaphoreType.DMA((1,)),
        ],
        compiler_params=pltpu.CompilerParams(vmem_limit_bytes=100 * 1024 * 1024),
    )(
        A_x[0].T, A_wqkv, A_wo, B_mem0[0],
        B_Wq.reshape(D * HB, DB), B_Wk.reshape(D * HB, DB), B_Wv.reshape(D * HB, DB),
        B_Wo.transpose(0, 2, 1).reshape(HB * D, DB), gate_w,
    )
    return outT.T[None]
```
